```python
import os as _os
_os.environ.setdefault("JAX_PLATFORMS", "cpu")
import jax
import jax.numpy as jnp

def _softmax(x, axis=-1):
    return jax.nn.softmax(x, axis=axis)
def _gelu(x):
    return jax.nn.gelu(x, approximate=True)
def _silu(x):
    return jax.nn.silu(x)
def _sigmoid(x):
    return jax.nn.sigmoid(x)
def _layernorm(x, axis=-1, eps=1e-5):
    m = jnp.mean(x, axis=axis, keepdims=True)
    v = jnp.var(x, axis=axis, keepdims=True)
    return (x - m) / jnp.sqrt(v + eps)
def _scatter_add(tgt, idx, src, axis=0):
    return tgt.at[idx].add(src)
def _segment_sum(src, seg, n):
    return jax.ops.segment_sum(src, seg, n)
class _Rng:
    def __init__(self, key):
        self._k = key
    def _next(self):
        self._k, sub = jax.random.split(self._k)
        return sub
    def normal(self, shape):
        return jax.random.normal(self._next(), shape, dtype=jnp.bfloat16)
    def randint(self, lo, hi, shape):
        return jax.random.randint(self._next(), shape, lo, hi, dtype=jnp.int32)
    def uniform(self, shape, lo=0.0, hi=1.0):
        return jax.random.uniform(self._next(), shape, jnp.bfloat16, lo, hi)
    def permutation(self, n):
        return jax.random.permutation(self._next(), n)


kernel_name = 'interleave_layers__sliding_local_dilated__sliding_local_dilated__prompt'

def setup_inputs():
    _rng = _Rng(jax.random.key(int.from_bytes(__import__("os").urandom(4), "little")))
    _w = (lambda a: (lambda t: t.astype(jnp.bfloat16) if jnp.issubdtype(t.dtype, jnp.floating) else t)(jnp.asarray(a)))
    def _A_setup():
        B, S, D = 1, 2048, 1024
        return {
            "x": _w((lambda *s: _rng.normal(s) * 0.05)(B, S, D)),
            "wqkv": _w((lambda *s: _rng.normal(s) * 0.05)(D, 3 * D)),
            "wo": _w((lambda *s: _rng.normal(s) * 0.05)(D, D)),
        }
    _A_in = _A_setup()

    def _B_setup():
        B, S, D = 1, 2048, 1024
        return {
            "x": _w((lambda *s: _rng.normal(s) * 0.05)(B, S, D)),
            "wqkv": _w((lambda *s: _rng.normal(s) * 0.05)(D, 3 * D)),
            "wo": _w((lambda *s: _rng.normal(s) * 0.05)(D, D)),
        }
    _B_in = _B_setup()

    return {
        "A_x": _A_in["x"],
        "A_wqkv": _A_in["wqkv"],
        "A_wo": _A_in["wo"],
        "B_x": _B_in["x"],
        "B_wqkv": _B_in["wqkv"],
        "B_wo": _B_in["wo"],
    }

def reference(A_x, A_wqkv, A_wo, B_x, B_wqkv, B_wo):
    def _A_ref(x, wqkv, wo):
        B, S, D = x.shape
        H = 32; Dh = D // H
        W, dil = 8, 2
        qkv = (lambda x, *d: x.transpose(*d))((x @ wqkv).reshape(B, S, 3, H, Dh), 2, 0, 3, 1, 4)
        q, k, v = qkv[0], qkv[1], qkv[2]
        scale = Dh ** -0.5
        pos = jnp.arange(S)
        off = jnp.arange(W) * dil
        idx = pos[:, None] - off[None, :]
        mask = idx >= 0
        idx_c = jnp.where(mask, idx, 0).reshape(-1)
        kg = k[:, :, idx_c, :].reshape(B, H, S, W, Dh)
        vg = v[:, :, idx_c, :].reshape(B, H, S, W, Dh)
        logits = jnp.einsum("bhsd,bhswd->bhsw", q, kg) * scale
        logits = jnp.where(mask[None, None, :, :], logits, -1e9)
        attn = _softmax(logits, axis=-1)
        o = jnp.einsum("bhsw,bhswd->bhsd", attn, vg)
        return (lambda x, *d: x.transpose(*d))(o, 0, 2, 1, 3).reshape(B, S, D) @ wo

    def _B_ref(x, wqkv, wo):
        B, S, D = x.shape
        H = 32; Dh = D // H
        W, dil = 8, 2
        qkv = (lambda x, *d: x.transpose(*d))((x @ wqkv).reshape(B, S, 3, H, Dh), 2, 0, 3, 1, 4)
        q, k, v = qkv[0], qkv[1], qkv[2]
        scale = Dh ** -0.5
        pos = jnp.arange(S)
        off = jnp.arange(W) * dil
        idx = pos[:, None] - off[None, :]
        mask = idx >= 0
        idx_c = jnp.where(mask, idx, 0).reshape(-1)
        kg = k[:, :, idx_c, :].reshape(B, H, S, W, Dh)
        vg = v[:, :, idx_c, :].reshape(B, H, S, W, Dh)
        logits = jnp.einsum("bhsd,bhswd->bhsw", q, kg) * scale
        logits = jnp.where(mask[None, None, :, :], logits, -1e9)
        attn = _softmax(logits, axis=-1)
        o = jnp.einsum("bhsw,bhswd->bhsd", attn, vg)
        return (lambda x, *d: x.transpose(*d))(o, 0, 2, 1, 3).reshape(B, S, D) @ wo

    x = A_x
    x = x + _A_ref(_layernorm(x, axis=-1), A_wqkv, A_wo)
    x = x + _B_ref(_layernorm(x, axis=-1), B_wqkv, B_wo)
    x = x + _A_ref(_layernorm(x, axis=-1), A_wqkv, A_wo)
    x = x + _B_ref(_layernorm(x, axis=-1), B_wqkv, B_wo)
    return x
```

```python
import functools

import jax
import jax.numpy as jnp
from jax import lax
from jax.experimental import pallas as pl
from jax.experimental.pallas import tpu as pltpu

S = 2048
D = 1024
DH = 32
WIN = 8
NG = 8
NCOL = 16
NCH = 4
CPC = NCOL // NCH
CW = CPC * 128
NEXT = 2 * WIN - 1
NLAYER = 4
ATT_PIECES = 32
LN_PIECES = D // 64 + 2 * (D // 32)
X_AHEAD = 3
OUT_PARTS = ((0, 768), (768, 256))
EPS = 1e-5
SCALE = DH ** -0.5
NEG = -1e9

F32 = jnp.float32
BF16 = jnp.bfloat16
U32 = jnp.uint32


def _to_words(v):
    return pltpu.bitcast(v, U32)


def _from_words(v):
    return pltpu.bitcast(v, BF16)


def _pack(lo, hi):
    return pltpu.bitcast(
        pltpu.pack_elementwise([lo, hi], packed_dtype=BF16), U32)


def _kernel(x_hbm, wa_hbm, woa_hbm, wb_hbm, wob_hbm, out_hbm,
            xio, xT, xn, oT, wraw, woraw, wt0, wt1, woT, wtmp,
            qa, ka, va, qb, kb, vb, sem_x, sem_w, sem_o):
    bufs = ((qa, ka, va), (qb, kb, vb))
    wts = (wt0, wt1)
    xio_words = xio.bitcast(U32)

    def x_copy(fb):
        return pltpu.make_async_copy(
            x_hbm.at[:, pl.ds(fb * 128, 128)], xio.at[fb], sem_x.at[fb])

    def out_copy(fb):
        return pltpu.make_async_copy(
            xio.at[fb], out_hbm.at[:, pl.ds(fb * 128, 128)], sem_o.at[fb])

    def w_copies(k):
        if k == 4:
            return [pltpu.make_async_copy(wb_hbm, wraw.at[1], sem_w.at[k]),
                    pltpu.make_async_copy(wob_hbm, woraw.at[1], sem_w.at[k])]
        g0, g1 = ((0, 1), (1, 2), (2, 4), (4, NG))[k]
        cps = []
        for sec in range(3):
            cols = pl.ds(sec * D + g0 * 128, (g1 - g0) * 128)
            cps.append(pltpu.make_async_copy(
                wa_hbm.at[:, cols], wraw.at[0, :, cols], sem_w.at[k]))
        if k >= 2:
            rows = pl.ds(0, 256) if k == 2 else pl.ds(256, D - 256)
            cps.append(pltpu.make_async_copy(
                woa_hbm.at[rows, :], woraw.at[0, rows, :], sem_w.at[k]))
        return cps

    def w_start(k):
        for cp in w_copies(k):
            cp.start()

    def w_wait(k):
        for cp in w_copies(k):
            cp.wait()

    def prep_wqkv(t, dst):
        s = (t // NG) % 2
        g = t % NG
        for sec in range(3):
            cols = pl.ds(pl.multiple_of(sec * D + g * 128, 128), 128)
            dst[pl.ds(sec * 64, 64), :] = _to_words(wraw[s, :, cols].T)

    def prep_wo(s, g):
        grp = pl.ds(pl.multiple_of(g * 128, 128), 128)
        for nt in range(D // 128):
            tile = woraw[s, grp, pl.ds(nt * 128, 128)].astype(F32)
            for h in range(4):
                wtmp[pl.ds(nt * 64 + h, 16, stride=4), :] = _pack(
                    tile[h * DH:h * DH + 16, :], tile[h * DH + 16:(h + 1) * DH, :])
        for nt in range(D // 128):
            woT[pl.ds(nt * 64, 64), grp] = _to_words(
                _from_words(wtmp[pl.ds(nt * 64, 64), :]).T)

    def drain(gen):
        for _ in gen:
            pass

    def chain(*gens):
        for gen in gens:
            yield from gen

    def pace(gen, pieces, tokens):
        next(gen, None)
        seen = [0]

        def side(token):
            seen[0] += 1
            if (seen[0] * pieces) // tokens > ((seen[0] - 1) * pieces) // tokens:
                try:
                    gen.send(token)
                except StopIteration:
                    pass
        return side

    def idle(token):
        del token

    def after(token, keep, val):
        return val if token is None else jnp.where(keep, val, token)

    def layernorm(col, keep):
        acc = [None] * 4
        for r in range(D // 64):
            tok = yield
            for j in range(8):
                blk = xT[col, pl.ds(r * 64 + j * 8, 8), :]
                if r == 0 and j < 4:
                    acc[j] = blk
                elif j < 4:
                    acc[j] = after(tok, keep, acc[j]) + blk
                else:
                    acc[j % 4] = acc[j % 4] + blk
        tot = (acc[0] + acc[1]) + (acc[2] + acc[3])
        mean = jnp.sum(tot, axis=0, keepdims=True) * (1.0 / D)
        mean = jnp.broadcast_to(mean, (8, 128))
        acc = [None] * 4
        for r in range(D // 32):
            mu = after((yield), keep, mean)
            for j in range(4):
                dv = xT[col, pl.ds(r * 32 + j * 8, 8), :] - mu
                acc[j] = dv * dv if r == 0 else acc[j] + dv * dv
        tot = (acc[0] + acc[1]) + (acc[2] + acc[3])
        var = jnp.sum(tot, axis=0, keepdims=True) * (1.0 / D)
        rstd = jnp.broadcast_to(lax.rsqrt(var + EPS), (8, 128))
        for r in range(D // 32):
            mu = after((yield), keep, mean)
            for j in range(2):
                r0 = r * 32 + j * 16
                ev = xT[col, pl.ds(r0, 8, stride=2), :]
                od = xT[col, pl.ds(r0 + 1, 8, stride=2), :]
                xn[col, pl.ds(r0 // 2, 8), :] = _pack(
                    (ev - mu) * rstd, (od - mu) * rstd)

    def split_dot(lhs_ref, rows, rhs_ref, side):
        half = jnp.dot(_from_words(lhs_ref[rows, pl.ds(0, D // 2)]),
                       _from_words(rhs_ref[pl.ds(0, D // 4), :]),
                       preferred_element_type=F32)
        for n in range(half.shape[0] // 8):
            side(half[n * 8:(n + 1) * 8, :])
        return half + jnp.dot(_from_words(lhs_ref[rows, pl.ds(D // 2, D // 2)]),
                              _from_words(rhs_ref[pl.ds(D // 4, D // 4), :]),
                              preferred_element_type=F32)

    def qkv_col(wt, buf, col, v_first, side):
        res = split_dot(wt, pl.ds(0, 192), xn.at[col], side)
        lane0 = lax.broadcasted_iota(jnp.int32, (8, 128), 1) == 0
        p, c = divmod(col, WIN)
        if col == 0:
            v_first = res[256:384, :]
        for sec in range(3):
            slot = col if sec == 0 else p * NEXT + WIN - 1 + c
            for h in range(4):
                for i in range(4):
                    r0 = h * DH + i * 8
                    t = res[sec * 128 + r0:sec * 128 + r0 + 8, :]
                    side(t)
                    dst = i * 32 + h
                    buf[sec][pl.ds(dst + slot * 128, 8, stride=4), :] = t
                    if sec > 0 and c > 0:
                        t = pltpu.roll(t, 1, 1)
                        if sec == 2:
                            t = jnp.where(lane0, v_first[r0:r0 + 8, :], t)
                        buf[sec][pl.ds(dst + (slot - WIN) * 128, 8, stride=4), :] = t
        return v_first

    def attend(buf, g, col, keep):
        p, c = divmod(col, WIN)
        base = p * NEXT + c
        lane0 = lax.broadcasted_iota(jnp.int32, (8, 128), 1) == 0

        def ld(sec, slot, i):
            return buf[sec][pl.ds(slot * 128 + i * 8, 8), :]

        acc = [[None] * WIN for _ in range(2)]
        for i in range(16):
            tok = yield
            qs = [after(tok, keep, ld(0, col + u, i)) for u in range(2)]
            for e in range(WIN + 1):
                kv = ld(1, base + e, i)
                for u in range(2):
                    w = WIN - 1 + u - e
                    if 0 <= w < WIN:
                        pr = qs[u] * kv
                        acc[u][w] = pr if i == 0 else acc[u][w] + pr
        prob = []
        for u in range(2):
            lg = []
            for w in range(WIN):
                a = acc[u][w]
                a = (a + pltpu.roll(a, 4, 0)) * SCALE
                if c + u - w < 0:
                    a = jnp.where(lane0, NEG, a)
                lg.append(a)
            m = lg[0]
            for w in range(1, WIN):
                m = jnp.maximum(m, lg[w])
            ex = [jnp.exp(a - m) for a in lg]
            den = ex[0]
            for w in range(1, WIN):
                den = den + ex[w]
            inv = 1.0 / den
            prob.append([e_ * inv for e_ in ex])
        for i2 in range(8):
            outs = [[], []]
            for i in (i2, i2 + 8):
                tok = yield
                o = [None, None]
                for e in range(WIN + 1):
                    vv = after(tok, keep, ld(2, base + e, i))
                    for u in range(2):
                        w = WIN - 1 + u - e
                        if 0 <= w < WIN:
                            pr = prob[u][w] * vv
                            o[u] = pr if o[u] is None else o[u] + pr
                for u in range(2):
                    outs[u].append(o[u])
            rows = pl.ds(pl.multiple_of(g * 64 + i2 * 8, 8), 8)
            for u in range(2):
                oT[col + u, rows, :] = _pack(*outs[u])

    def attend_all(buf, g, keep, first=0):
        return chain(*[attend(buf, g, col, keep)
                       for col in range(first, NCOL, 2)])

    def out_col(col, r0, nr, side):
        res = split_dot(woT, pl.ds(r0 // 2, nr // 2), oT.at[col], side)
        for r in range(nr // 8):
            rows = pl.ds(r0 + r * 8, 8)
            t = res[r * 8:(r + 1) * 8, :]
            side(t)
            xT[col, rows, :] = xT[col, rows, :] + t

    def emit(c, r0, nr, keep):
        for fb in range(r0 // 128, (r0 + nr) // 128):
            words = []
            for r in range(16):
                if r % 4 == 0:
                    tok = yield
                rows = pl.ds(fb * 128 + r * 8, 8)
                words.append(_pack(after(tok, keep, xT[c, rows, :]),
                                   xT[WIN + c, rows, :]))
            xio_words[fb, pl.ds(c, 128, stride=8), :] = (
                jnp.concatenate(words, axis=0).T)

    nfb = D // 128
    w_start(0)
    for fb in range(X_AHEAD):
        x_copy(fb).start()
    w_wait(0)
    prep_wqkv(0, wt0)
    for fb in range(nfb):
        x_copy(fb).wait()
        if fb + X_AHEAD < nfb:
            x_copy(fb + X_AHEAD).start()
        elif fb == nfb - 2:
            w_start(1)
        for c in range(WIN):
            wd = xio_words[fb, pl.ds(c, 128, stride=8), :].T
            for p in range(2):
                bits = (wd << 16) if p == 0 else (wd & jnp.uint32(0xFFFF0000))
                xT[p * WIN + c, pl.ds(fb * 128, 128), :] = (
                    pltpu.bitcast(bits, F32))
    drain(layernorm(0, None))
    drain(layernorm(1, None))
    w_wait(1)
    w_start(2)

    def step(layer, g, par, keep):
        first = isinstance(g, int) and g == 0
        last = isinstance(g, int) and g == NG - 1
        tokens = 2 * 384 // 8
        if first:
            att = chain(*[layernorm(col, keep) for col in range(2, NCOL)])
            side = pace(att, LN_PIECES, tokens)
        else:
            work = [attend(bufs[1 - par], g - 1, col, keep)
                    for col in range(0, NCOL, 2)]
            if last:
                work.append(attend(bufs[par], g, 0, keep))
            att = chain(*work)
            side = pace(att, ATT_PIECES * len(work), tokens * (NCOL - 1))
        v_first = None
        for col in range(NCOL):
            v_first = qkv_col(wts[par], bufs[par], col, v_first, side)
            if col == 4:
                prep_wqkv(layer * NG + g + 1, wts[1 - par])
            if col == 9 and not first:
                prep_wo(layer % 2, g - 1)
            if col == 12 and last:
                prep_wo(layer % 2, g)
        drain(att)

    def project_out(layer, keep):
        r0, nr = OUT_PARTS[0]
        tokens = 2 * nr // 8
        order = [0, 1, WIN, WIN + 1] + [
            p * WIN + c for c in range(2, WIN) for p in range(2)]
        att = chain(*[attend(bufs[1], NG - 1, p * WIN + c, keep)
                      for c in range(0, WIN, 2) for p in range(2)][1:])
        att_side = pace(att, ATT_PIECES, tokens)
        todo, todo_side = iter(()), idle
        for n, col in enumerate(order):
            out_col(col, r0, nr, lambda t: (att_side(t), todo_side(t)))
            if n >= 3 and n % 2 == 1:
                drain(todo)
                done = (0, 1) if n == 3 else (col - WIN,)
                todo = chain(*[emit(c, r0, nr, keep) for c in done])
                if n + 1 < NCOL:
                    todo_side = pace(todo, len(done) * nr // 32, 2 * tokens)
        drain(att)

        pieces = nr // 32
        r0, nr = OUT_PARTS[1]
        tokens = 2 * nr // 8
        todo_side = pace(todo, pieces, 3 * tokens)
        order = [p * WIN + c for c in range(WIN) for p in range(2)]
        for n, col in enumerate(order):
            out_col(col, r0, nr, todo_side)
            if n == 3:
                drain(todo)

                @pl.loop(0, (layer == NLAYER - 1).astype(jnp.int32))
                def _(i):
                    for fb in range(r0 // 128):
                        out_copy(fb).start()
                todo = chain(emit(0, r0, nr, keep), emit(1, r0, nr, keep),
                             layernorm(0, keep), layernorm(1, keep))
                todo_side = pace(todo, 2 * (nr // 32 + LN_PIECES), 4 * tokens)
            elif n >= 7 and n % 2 == 1:
                drain(todo)
                done = (2, 3) if n == 7 else (col - WIN,)
                todo = chain(*[emit(c, r0, nr, keep) for c in done])
                if n + 1 < NCOL:
                    todo_side = pace(todo, len(done) * nr // 32, tokens)
        drain(todo)

    def layer_body(layer, carry):
        keep = lax.broadcasted_iota(jnp.int32, (8, 128), 1) >= layer - NLAYER
        step(layer, 0, 0, keep)

        @pl.when(layer == 0)
        def _():
            w_wait(2)
            w_start(3)

        def pair(i, c2):
            @pl.when(jnp.logical_and(layer == 0, i == 1))
            def _():
                w_wait(3)
                w_start(4)
            step(layer, 2 * i + 1, 1, keep)
            step(layer, 2 * i + 2, 0, keep)
            return c2
        lax.fori_loop(0, NG // 2 - 1, pair, 0)

        @pl.when(layer == 0)
        def _():
            w_wait(4)
        step(layer, NG - 1, 1, keep)
        project_out(layer, keep)
        return carry

    lax.fori_loop(0, NLAYER, layer_body, 0)

    for fb in range(OUT_PARTS[0][1] // 128, nfb):
        out_copy(fb).start()
    for fb in range(nfb):
        out_copy(fb).wait()


@jax.jit
def pallas_interleave_layers__sliding_local_dilated__sliding_local_dilated__prompt_kernel(
    A_x: jax.Array,
    A_wqkv: jax.Array,
    A_wo: jax.Array,
    B_x: jax.Array,
    B_wqkv: jax.Array,
    B_wo: jax.Array,
):
    del B_x
    any_spec = pl.BlockSpec(memory_space=pl.ANY)
    qbuf = pltpu.VMEM((NCOL * 128, 128), F32)
    kvbuf = pltpu.VMEM((2 * NEXT * 128, 128), F32)
    out = pl.pallas_call(
        _kernel,
        out_shape=jax.ShapeDtypeStruct((S, D), BF16),
        in_specs=[any_spec] * 5,
        out_specs=any_spec,
        scratch_shapes=[
            pltpu.VMEM((D // 128, S, 128), BF16),
            pltpu.VMEM((NCOL, D, 128), F32),
            pltpu.VMEM((NCOL, D // 2, 128), U32),
            pltpu.VMEM((NCOL, D // 2, 128), U32),
            pltpu.VMEM((2, D, 3 * D), BF16),
            pltpu.VMEM((2, D, D), BF16),
            pltpu.VMEM((192, D), U32),
            pltpu.VMEM((192, D), U32),
            pltpu.VMEM((D // 2, D), U32),
            pltpu.VMEM((D // 2, 128), U32),
            qbuf, kvbuf, kvbuf, qbuf, kvbuf, kvbuf,
            pltpu.SemaphoreType.DMA((D // 128,)),
            pltpu.SemaphoreType.DMA((5,)),
            pltpu.SemaphoreType.DMA((D // 128,)),
        ],
        compiler_params=pltpu.CompilerParams(
            vmem_limit_bytes=100 * 1024 * 1024),
    )(A_x.reshape(S, D), A_wqkv, A_wo, B_wqkv, B_wo)
    return out.reshape(1, S, D)
```

```python
import functools

import jax
import jax.numpy as jnp
from jax import lax
from jax.experimental import pallas as pl
from jax.experimental.pallas import tpu as pltpu

S = 2048
D = 1024
DH = 32
WIN = 8
NG = 8
NCOL = 16
NEXT = 2 * WIN - 1
NLAYER = 4
PAD = 8
QKV_ORDER = tuple(range(WIN)) + tuple(range(WIN + 1, NCOL)) + (WIN,)
ATT_PIECES = 32
LN_PIECES = D // 64 + 2 * (D // 32)
OUT_PARTS = ((0, 512), (512, 384), (896, 128))
EPS = 1e-5
SCALE = DH ** -0.5
NEG = -1e9

F32 = jnp.float32
BF16 = jnp.bfloat16
U32 = jnp.uint32


def _to_words(v):
    return pltpu.bitcast(v, U32)


def _from_words(v):
    return pltpu.bitcast(v, BF16)


def _pack(lo, hi):
    lo = pltpu.bitcast(lo.astype(BF16).astype(F32), U32)
    hi = pltpu.bitcast(hi.astype(BF16).astype(F32), U32)
    return (lo >> 16) | hi


def _only_if(cond):
    def run(body):
        pl.loop(0, cond.astype(jnp.int32))(lambda _: body())
    return run


def _kernel(x_hbm, wa_hbm, woa_hbm, wb_hbm, wob_hbm, out_hbm,
            xio, xT, xn, oT, wraw, woraw, wt0, wt1, woT, wtmp,
            qa, ka, va, qb, kb, vb, sem_x, sem_w, sem_o):
    bufs = ((qa, ka, va), (qb, kb, vb))
    wts = (wt0, wt1)
    xio_words = xio.bitcast(U32)

    def x_copy(fb):
        return pltpu.make_async_copy(
            x_hbm.at[:, pl.ds(fb * 128, 128)], xio.at[fb, pl.ds(0, S)],
            sem_x.at[fb])

    def out_copy(fb):
        return pltpu.make_async_copy(
            xio.at[fb, pl.ds(0, S)], out_hbm.at[:, pl.ds(fb * 128, 128)],
            sem_o.at[fb])

    def w_copies(k):
        if k == 3:
            return [pltpu.make_async_copy(wb_hbm, wraw.at[1], sem_w.at[k]),
                    pltpu.make_async_copy(wob_hbm, woraw.at[1], sem_w.at[k])]
        g0, g1 = ((0, 1), (1, 4), (4, NG))[k]
        cps = []
        for sec in range(3):
            cols = pl.ds(sec * D + g0 * 128, (g1 - g0) * 128)
            cps.append(pltpu.make_async_copy(
                wa_hbm.at[:, cols], wraw.at[0, :, cols], sem_w.at[k]))
        if k >= 1:
            rows = pl.ds(0, 256) if k == 1 else pl.ds(256, D - 256)
            cps.append(pltpu.make_async_copy(
                woa_hbm.at[rows, :], woraw.at[0, rows, :], sem_w.at[k]))
        return cps

    def w_start(k):
        for cp in w_copies(k):
            cp.start()

    def w_wait(k):
        for cp in w_copies(k):
            cp.wait()

    def prep_wqkv(t, dst):
        s = (t // NG) % 2
        g = t % NG
        for sec in range(3):
            cols = pl.ds(pl.multiple_of(sec * D + g * 128, 128), 128)
            dst[pl.ds(sec * 64, 64), :] = _to_words(wraw[s, :, cols].T)

    def prep_wo(s, g):
        grp = pl.ds(pl.multiple_of(g * 128, 128), 128)
        for nt in range(D // 128):
            tile = woraw[s, grp, pl.ds(nt * 128, 128)].astype(F32)
            for h in range(4):
                wtmp[pl.ds(nt * 64 + h, 16, stride=4), :] = _pack(
                    tile[h * DH:h * DH + 16, :],
                    tile[h * DH + 16:(h + 1) * DH, :])
        for nt in range(D // 128):
            woT[pl.ds(nt * 64, 64), grp] = _to_words(
                _from_words(wtmp[pl.ds(nt * 64, 64), :]).T)

    def drain(gen):
        for _ in gen:
            pass

    def chain(*gens):
        for gen in gens:
            yield from gen

    def pace(gen, pieces, tokens):
        next(gen, None)
        seen = [0]

        def side(token):
            seen[0] += 1
            if (seen[0] * pieces) // tokens > ((seen[0] - 1) * pieces) // tokens:
                try:
                    gen.send(token)
                except StopIteration:
                    pass
        return side

    def idle(token):
        del token

    def after(token, keep, val):
        return val if token is None else jnp.where(keep, val, token)

    def layernorm(col, keep):
        acc = [None] * 4
        for r in range(D // 64):
            tok = yield
            for j in range(8):
                blk = xT[col, pl.ds(r * 64 + j * 8, 8), :]
                if r == 0 and j < 4:
                    acc[j] = blk
                elif j < 4:
                    acc[j] = after(tok, keep, acc[j]) + blk
                else:
                    acc[j % 4] = acc[j % 4] + blk
        tot = (acc[0] + acc[1]) + (acc[2] + acc[3])
        mean = jnp.sum(tot, axis=0, keepdims=True) * (1.0 / D)
        mean = jnp.broadcast_to(mean, (8, 128))
        acc = [None] * 4
        for r in range(D // 32):
            mu = after((yield), keep, mean)
            for j in range(4):
                dv = xT[col, pl.ds(r * 32 + j * 8, 8), :] - mu
                acc[j] = dv * dv if r == 0 else acc[j] + dv * dv
        tot = (acc[0] + acc[1]) + (acc[2] + acc[3])
        var = jnp.sum(tot, axis=0, keepdims=True) * (1.0 / D)
        rstd = jnp.broadcast_to(lax.rsqrt(var + EPS), (8, 128))
        for r in range(D // 32):
            mu = after((yield), keep, mean)
            for j in range(2):
                r0 = r * 32 + j * 16
                ev = xT[col, pl.ds(r0, 8, stride=2), :]
                od = xT[col, pl.ds(r0 + 1, 8, stride=2), :]
                xn[col, pl.ds(r0 // 2, 8), :] = _pack(
                    (ev - mu) * rstd, (od - mu) * rstd)

    def split_dot(lhs_ref, rows, rhs_ref, side, gate=None):
        rhs = rhs_ref[pl.ds(0, D // 4), :]
        if gate is not None:
            rhs = jnp.concatenate([gate(rhs[:8, :]), rhs[8:, :]], axis=0)
        half = jnp.dot(_from_words(lhs_ref[rows, pl.ds(0, D // 2)]),
                       _from_words(rhs), preferred_element_type=F32)
        for n in range(half.shape[0] // 8):
            side(half[n * 8:(n + 1) * 8, :])
        return half + jnp.dot(_from_words(lhs_ref[rows, pl.ds(D // 2, D // 2)]),
                              _from_words(rhs_ref[pl.ds(D // 4, D // 4), :]),
                              preferred_element_type=F32)

    def qkv_col(wt, buf, col, v_first, side):
        res = split_dot(wt, pl.ds(0, 192), xn.at[col], side)
        lane0 = lax.broadcasted_iota(jnp.int32, (8, 128), 1) == 0
        p, c = divmod(col, WIN)
        if col == 0:
            v_first = res[256:384, :]
        for sec in range(3):
            slot = col if sec == 0 else p * NEXT + WIN - 1 + c
            for h in range(4):
                for i in range(4):
                    r0 = h * DH + i * 8
                    t = res[sec * 128 + r0:sec * 128 + r0 + 8, :]
                    side(t)
                    dst = i * 32 + h
                    buf[sec][pl.ds(dst + slot * 128, 8, stride=4), :] = t
                    if sec > 0 and c > 0:
                        t = pltpu.roll(t, 1, 1)
                        if sec == 2:
                            t = jnp.where(lane0, v_first[r0:r0 + 8, :], t)
                        shifted = dst + (slot - WIN) * 128
                        buf[sec][pl.ds(shifted, 8, stride=4), :] = t
        return v_first

    def attend(buf, g, col, keep):
        p, c = divmod(col, WIN)
        base = p * NEXT + c
        lane0 = lax.broadcasted_iota(jnp.int32, (8, 128), 1) == 0

        def ld(sec, slot, i):
            return buf[sec][pl.ds(slot * 128 + i * 8, 8), :]

        acc = [[None] * WIN for _ in range(2)]
        for i in range(16):
            tok = yield
            qs = [after(tok, keep, ld(0, col + u, i)) for u in range(2)]
            for e in range(WIN + 1):
                kv = ld(1, base + e, i)
                for u in range(2):
                    w = WIN - 1 + u - e
                    if 0 <= w < WIN:
                        pr = qs[u] * kv
                        acc[u][w] = pr if i == 0 else acc[u][w] + pr
        prob = []
        for u in range(2):
            lg = []
            for w in range(WIN):
                a = acc[u][w]
                a = (a + pltpu.roll(a, 4, 0)) * SCALE
                if c + u - w < 0:
                    a = jnp.where(lane0, NEG, a)
                lg.append(a)
            m = lg[0]
            for w in range(1, WIN):
                m = jnp.maximum(m, lg[w])
            ex = [jnp.exp(a - m) for a in lg]
            den = ex[0]
            for w in range(1, WIN):
                den = den + ex[w]
            inv = 1.0 / den
            prob.append([e_ * inv for e_ in ex])
        for i2 in range(8):
            outs = [[], []]
            for i in (i2, i2 + 8):
                tok = yield
                o = [None, None]
                for e in range(WIN + 1):
                    vv = after(tok, keep, ld(2, base + e, i))
                    for u in range(2):
                        w = WIN - 1 + u - e
                        if 0 <= w < WIN:
                            pr = prob[u][w] * vv
                            o[u] = pr if o[u] is None else o[u] + pr
                for u in range(2):
                    outs[u].append(o[u])
            rows = pl.ds(pl.multiple_of(g * 64 + i2 * 8, 8), 8)
            for u in range(2):
                oT[col + u, rows, :] = _pack(*outs[u])

    def out_col(col, r0, nr, side, gate=None):
        res = split_dot(woT, pl.ds(r0 // 2, nr // 2), oT.at[col], side, gate)
        for r in range(nr // 8):
            rows = pl.ds(r0 + r * 8, 8)
            t = res[r * 8:(r + 1) * 8, :]
            side(t)
            xT[col, rows, :] = xT[col, rows, :] + t

    def emit(c, r0, nr, keep):
        for fb in range(r0 // 128, (r0 + nr) // 128):
            words = []
            for r in range(16):
                if r % 4 == 0:
                    tok = yield
                rows = pl.ds(fb * 128 + r * 8, 8)
                words.append(_pack(after(tok, keep, xT[c, rows, :]),
                                   xT[WIN + c, rows, :]))
            xio_words[fb, pl.ds(c, 128, stride=8), :] = (
                jnp.concatenate(words, axis=0).T)

    nfb = D // 128
    for fb in range(nfb):
        x_copy(fb).start()
    w_start(0)

    @pl.loop(0, nfb)
    def _(fb):
        x_copy(fb).wait()
        rows = pl.ds(pl.multiple_of(fb * 128, 128), 128)
        for c in range(WIN):
            wd = xio_words[fb, pl.ds(c, 128, stride=8), :].T
            for p in range(2):
                bits = (wd << 16) if p == 0 else (wd & jnp.uint32(0xFFFF0000))
                xT[p * WIN + c, rows, :] = pltpu.bitcast(bits, F32)
    drain(layernorm(0, None))
    w_wait(0)
    w_start(1)
    prep_wqkv(0, wt0)

    def step(layer, g, par, keep):
        first = isinstance(g, int) and g == 0
        last = isinstance(g, int) and g == NG - 1
        tokens = 2 * 384 // 8
        if first:
            att = chain(*[layernorm(col, keep) for col in QKV_ORDER[1:]])
            side = pace(att, LN_PIECES * (NCOL - 1), tokens * (NCOL - 4))
        else:
            work = [attend(bufs[1 - par], g - 1, col, keep)
                    for col in range(0, NCOL, 2)]
            if last:
                work.append(attend(bufs[par], g, 0, keep))
            att = chain(*work)
            side = pace(att, ATT_PIECES * len(work), tokens * (NCOL - 3))
        v_first = None
        for col in QKV_ORDER:
            v_first = qkv_col(wts[par], bufs[par], col, v_first, side)
            if col == 4 and not first:
                prep_wqkv(layer * NG + g + 1, wts[1 - par])
            if col == 9 and not first:
                prep_wo(layer % 2, g - 1)
            if col == 12 and last:
                prep_wo(layer % 2, g)
        drain(att)

    def project_out(layer, keep):
        order = [0, 1, WIN, WIN + 1] + [
            p * WIN + c for c in range(2, WIN) for p in range(2)]
        att = chain(*[attend(bufs[1], NG - 1, p * WIN + c, keep)
                      for c in range(0, WIN, 2) for p in range(2)][1:])
        att_side = pace(att, ATT_PIECES, 2 * OUT_PARTS[0][1] // 8)
        todo, pieces, gate = iter(()), 0, None
        for part, (r0, nr) in enumerate(OUT_PARTS):
            tokens = 2 * nr // 8
            todo_side = pace(todo, pieces, tokens)
            for n, col in enumerate(order):
                out_col(col, r0, nr, lambda t: (att_side(t), todo_side(t)),
                        gate if n == 3 else None)
                if part == 0 and n == 10:
                    prep_wqkv((layer + 1) * NG + 1, wts[1])
                if part > 0 and n == 1:
                    drain(todo)
                    p0, pn = OUT_PARTS[part - 1]

                    @pl.when(layer == NLAYER - 1)
                    def _():
                        for fb in range(p0 // 128, (p0 + pn) // 128):
                            out_copy(fb).start()
                    spare = pl.ds(S // 2, PAD)
                    xio_words[nfb - 1 + layer // NLAYER, spare, :] = (
                        jnp.zeros((PAD, 128), U32))
                    gate = functools.partial(
                        after,
                        xio_words[nfb - 1 + layer // (NLAYER + 1), spare, :],
                        keep)
                if n >= 3 and n % 2 == 1:
                    drain(todo)
                    done = (0, 1) if n == 3 else (col - WIN,)
                    work = [emit(c, r0, nr, keep) for c in done]
                    pieces = len(done) * nr // 32
                    todo = chain(*work)
                    if n + 1 < NCOL:
                        todo_side = pace(todo, pieces, tokens)
                if part == len(OUT_PARTS) - 1 and n == 0:
                    att = layernorm(0, keep)
                    att_side = pace(att, LN_PIECES, 8 * tokens)
            drain(att)
        drain(todo)

    def layer_body(layer, carry):
        keep = lax.broadcasted_iota(jnp.int32, (8, 128), 1) >= layer - NLAYER
        step(layer, 0, 0, keep)

        @_only_if(layer == 0)
        def _():
            w_wait(1)
            w_start(2)
            w_start(3)
            prep_wqkv(1, wts[1])

        def pair(i, c2):
            @pl.when(jnp.logical_and(layer == 0, i == 1))
            def _():
                w_wait(2)
            step(layer, 2 * i + 1, 1, keep)
            step(layer, 2 * i + 2, 0, keep)
            return c2
        lax.fori_loop(0, NG // 2 - 1, pair, 0)

        @pl.when(layer == 0)
        def _():
            w_wait(3)
        step(layer, NG - 1, 1, keep)
        project_out(layer, keep)
        return carry

    lax.fori_loop(0, NLAYER, layer_body, 0)

    for fb in range(OUT_PARTS[-1][0] // 128, nfb):
        out_copy(fb).start()
    for fb in range(nfb):
        out_copy(fb).wait()


@jax.jit
def pallas_interleave_layers__sliding_local_dilated__sliding_local_dilated__prompt_kernel(
    A_x: jax.Array,
    A_wqkv: jax.Array,
    A_wo: jax.Array,
    B_x: jax.Array,
    B_wqkv: jax.Array,
    B_wo: jax.Array,
):
    del B_x
    any_spec = pl.BlockSpec(memory_space=pl.ANY)
    qbuf = pltpu.VMEM((NCOL * 128 + PAD, 128), F32)
    kvbuf = pltpu.VMEM((2 * NEXT * 128 + PAD, 128), F32)
    out = pl.pallas_call(
        _kernel,
        out_shape=jax.ShapeDtypeStruct((S, D), BF16),
        in_specs=[any_spec] * 5,
        out_specs=any_spec,
        scratch_shapes=[
            pltpu.VMEM((D // 128, S + 2 * PAD, 128), BF16),
            pltpu.VMEM((NCOL, D + PAD, 128), F32),
            pltpu.VMEM((NCOL, D // 2, 128), U32),
            pltpu.VMEM((NCOL, D // 2, 128), U32),
            pltpu.VMEM((2, D, 3 * D), BF16),
            pltpu.VMEM((2, D, D), BF16),
            pltpu.VMEM((192, D), U32),
            pltpu.VMEM((192, D), U32),
            pltpu.VMEM((D // 2, D), U32),
            pltpu.VMEM((D // 2 + PAD, 128), U32),
            qbuf, kvbuf, kvbuf, qbuf, kvbuf, kvbuf,
            pltpu.SemaphoreType.DMA((D // 128,)),
            pltpu.SemaphoreType.DMA((4,)),
            pltpu.SemaphoreType.DMA((D // 128,)),
        ],
        compiler_params=pltpu.CompilerParams(
            vmem_limit_bytes=100 * 1024 * 1024),
    )(A_x.reshape(S, D), A_wqkv, A_wo, B_wqkv, B_wo)
    return out.reshape(1, S, D)
```
